```python
import jax
import jax.numpy as jnp

def _softmax(x, axis=-1):
    return jax.nn.softmax(x, axis=axis)
def _gelu(x):
    return jax.nn.gelu(x, approximate=True)
def _silu(x):
    return jax.nn.silu(x)
def _sigmoid(x):
    return jax.nn.sigmoid(x)
def _layernorm(x, axis=-1, eps=1e-5):
    m = jnp.mean(x, axis=axis, keepdims=True)
    v = jnp.var(x, axis=axis, keepdims=True)
    return (x - m) / jnp.sqrt(v + eps)
def _scatter_add(tgt, idx, src, axis=0):
    return tgt.at[idx].add(src)
def _segment_sum(src, seg, n):
    return jax.ops.segment_sum(src, seg, n)
class _Rng:
    def __init__(self, key):
        self._k = key
    def _next(self):
        self._k, sub = jax.random.split(self._k)
        return sub
    def normal(self, shape):
        return jax.random.normal(self._next(), shape, dtype=jnp.bfloat16)
    def randint(self, lo, hi, shape):
        return jax.random.randint(self._next(), shape, lo, hi, dtype=jnp.int32)
    def uniform(self, shape, lo=0.0, hi=1.0):
        return jax.random.uniform(self._next(), shape, jnp.bfloat16, lo, hi)
    def permutation(self, n):
        return jax.random.permutation(self._next(), n)


kernel_name = 'sequential_preLN__compressed_kv_cla__moe_arch_mod__prompt'

def setup_inputs():
    _rng = _Rng(jax.random.key(int.from_bytes(__import__("os").urandom(4), "little")))
    _w = (lambda a: (lambda t: t.astype(jnp.bfloat16) if jnp.issubdtype(t.dtype, jnp.floating) else t)(jnp.asarray(a)))
    def _A_setup():
        B, H, Sq, Sk, D, M = 1, 32, 2048, 2048, 128, 1024
        Dc = 4 * D
        return {
            "x": _w((lambda *s: _rng.normal(s) * 0.05)(B, Sq, M)),
            "c_kv": _w((lambda *s: _rng.normal(s) * 0.05)(B, Sk, Dc)),
            "w_q": _w((lambda *s: _rng.normal(s) * 0.05)(M, H, D) * (M ** -0.5)),
            "w_uk": _w((lambda *s: _rng.normal(s) * 0.05)(Dc, H, D) * (Dc ** -0.5)),
            "w_uv": _w((lambda *s: _rng.normal(s) * 0.05)(Dc, H, D) * (Dc ** -0.5)),
            "w_o": _w((lambda *s: _rng.normal(s) * 0.05)(H, D, M) * ((H * D) ** -0.5)),
        }
    _A_in = _A_setup()

    def _B_setup():
        B, S, D, F, C = 1, 2048, 1024, 3584, 2
        return {
            "x": _w((lambda *s: _rng.normal(s) * 0.05)(B, S, D)),
            "w_r": _w((lambda *s: _rng.normal(s) * 0.05)(D)),
            "w_gate": _w((lambda *s: _rng.normal(s) * 0.05)(D, F)),
            "w_up": _w((lambda *s: _rng.normal(s) * 0.05)(D, F)),
            "w_down": _w((lambda *s: _rng.normal(s) * 0.05)(F, D)),
        }
    _B_in = _B_setup()

    return {
        "A_x": _A_in["x"],
        "A_c_kv": _A_in["c_kv"],
        "A_w_q": _A_in["w_q"],
        "A_w_uk": _A_in["w_uk"],
        "A_w_uv": _A_in["w_uv"],
        "A_w_o": _A_in["w_o"],
        "B_x": _B_in["x"],
        "B_w_r": _B_in["w_r"],
        "B_w_gate": _B_in["w_gate"],
        "B_w_up": _B_in["w_up"],
        "B_w_down": _B_in["w_down"],
    }

def reference(A_x, A_c_kv, A_w_q, A_w_uk, A_w_uv, A_w_o, B_x, B_w_r, B_w_gate, B_w_up, B_w_down):
    def _A_ref(x, c_kv, w_q, w_uk, w_uv, w_o):
        B, Sq, M = x.shape[0], x.shape[1], x.shape[2]
        Sk = c_kv.shape[1]
        H, D = w_q.shape[1], w_q.shape[2]
        q = jnp.einsum("bqm,mhd->bhqd", x, w_q)
        k = jnp.einsum("bkc,chd->bhkd", c_kv, w_uk)
        v = jnp.einsum("bkc,chd->bhkd", c_kv, w_uv)
        scores = jnp.einsum("bhqd,bhkd->bhqk", q, k) * (D ** -0.5)
        off = Sk - Sq
        qi = jnp.arange(Sq)[:, None]
        kj = jnp.arange(Sk)[None, :]
        cmask = kj <= (qi + off)
        scores = jnp.where(cmask[None, None], scores, -1e9)
        p = _softmax(scores, axis=-1)
        ctx = jnp.einsum("bhqk,bhkd->bhqd", p, v)
        return jnp.einsum("bhqd,hdm->bqm", ctx, w_o)

    def _B_ref(x, w_r, w_gate, w_up, w_down):
        B, S, D = x.shape
        C = 2
        r = x @ w_r
        idx = jnp.argsort(-r, axis=-1)[:, :C]
        idx_e = jnp.repeat(idx.reshape(B, C, 1), D, axis=2)
        x_sel = jnp.take_along_axis(x, idx_e, axis=1)
        g = _silu(x_sel @ w_gate)
        u = x_sel @ w_up
        y = (g * u) @ w_down
        r_sel = _sigmoid(jnp.take_along_axis(r, idx, axis=1))
        y = y * r_sel.reshape(B, C, 1)
        b_off = (jnp.arange(B) * S).reshape(B, 1)
        flat_idx = (idx + b_off).reshape(B * C)
        zero = (x * 0.0).reshape(B * S, D)
        upd = _scatter_add(zero, flat_idx, y.reshape(B * C, D), axis=0)
        return x + upd.reshape(B, S, D)

    x = A_x
    h = x + _A_ref(_layernorm(x, axis=-1), A_c_kv, A_w_q, A_w_uk, A_w_uv, A_w_o)
    h2 = h + _B_ref(_layernorm(h, axis=-1), B_w_r, B_w_gate, B_w_up, B_w_down)
    return h2
```

```python
import functools
import math

import jax
import jax.numpy as jnp
from jax import lax
import jax.experimental.pallas as pl
import jax.experimental.pallas.tpu as pltpu

F32 = jnp.float32
BF16 = jnp.bfloat16
EPS = 1e-5
BQ = 256
RB = 256
NPAIRS = 16
GROUP = 4
NT = (((1,), (1,)), ((), ()))


def _layernorm(x):
    m = jnp.mean(x, axis=-1, keepdims=True)
    d = x - m
    v = jnp.mean(d * d, axis=-1, keepdims=True)
    return d * lax.rsqrt(v + EPS)


def _relayout(w_ref, dst_ref, g, c, rows):
    m0 = pl.multiple_of(c * rows, rows)
    base = pl.multiple_of(m0 * NPAIRS + g * GROUP, GROUP)
    win = w_ref.bitcast(jnp.uint32).at[pl.ds(base, (rows - 1) * NPAIRS + GROUP), :]
    for s in range(GROUP):
        u = win[pl.ds(s, rows, stride=NPAIRS), :]
        lo = pltpu.bitcast(u << 16, F32).astype(BF16)
        hi = pltpu.bitcast(u & jnp.uint32(0xFFFF0000), F32).astype(BF16)
        dst_ref[g * GROUP + s, pl.ds(m0, rows), :] = jnp.concatenate([lo, hi], axis=1)


def _kernel(x_hbm, ckv_hbm, wq_hbm, wuk_hbm, wuv_hbm, wo_hbm, wr_ref, wg_hbm, wu_hbm, wd_hbm, out_ref,
            x_v, ckv_v, wq_v, wuk_v, wuv_v, wo_v, wg_v, wu_v, wd_v,
            wq2_v, wuk2_v, wuv2_v, xn_v, q_v, k_v, v_v, ctx_v, r_v, sems, *, S, M, H, D, Dc):
    npairs = H // 2
    cp = lambda i, s, d: pltpu.make_async_copy(s, d, sems.at[i])
    c_x, c_ckv, c_wq = cp(0, x_hbm, x_v), cp(1, ckv_hbm, ckv_v), cp(2, wq_hbm, wq_v)
    c_wuk, c_wuv, c_wo = cp(3, wuk_hbm, wuk_v), cp(4, wuv_hbm, wuv_v), cp(5, wo_hbm, wo_v)
    c_wg, c_wu, c_wd = cp(6, wg_hbm, wg_v), cp(7, wu_hbm, wu_v), cp(8, wd_hbm, wd_v)
    for c in (c_x, c_wq, c_ckv, c_wuk, c_wuv):
        c.start()
    c_x.wait()

    def ln1(b, _):
        rows = pl.ds(pl.multiple_of(b * RB, RB), RB)
        xn_v[rows, :] = _layernorm(x_v[rows, :].astype(F32)).astype(BF16)
        return 0
    lax.fori_loop(0, S // RB, ln1, 0)
    c_wq.wait(); c_ckv.wait(); c_wuk.wait(); c_wuv.wait()
    for c in (c_wo, c_wg, c_wu, c_wd):
        c.start()

    qscale = (D ** -0.5) * math.log2(math.e)
    nq = S // BQ

    def attend(e, h):
        ri = lax.broadcasted_iota(jnp.int32, (BQ, BQ), 0)
        ci = lax.broadcasted_iota(jnp.int32, (BQ, BQ), 1)
        for i in range(nq):
            r0 = i * BQ
            q = q_v[e, r0:r0 + BQ, :]
            sd = lax.dot_general(q, k_v[e, r0:r0 + BQ, :], NT, preferred_element_type=F32)
            sd = jnp.where(ci <= ri, sd, -1e9)
            m = jnp.max(sd, axis=1, keepdims=True)
            if i > 0:
                so = lax.dot_general(q, k_v[e, 0:r0, :], NT, preferred_element_type=F32)
                m = jnp.maximum(m, jnp.max(so, axis=1, keepdims=True))
            pd = jnp.exp2(sd - m)
            l = jnp.sum(pd, axis=1, keepdims=True)
            o = jnp.dot(pd.astype(BF16), v_v[e, r0:r0 + BQ, :], preferred_element_type=F32)
            if i > 0:
                po = jnp.exp2(so - m)
                l = l + jnp.sum(po, axis=1, keepdims=True)
                o = o + jnp.dot(po.astype(BF16), v_v[e, 0:r0, :], preferred_element_type=F32)
            ctx_v[h, r0:r0 + BQ, :] = (o / l).astype(BF16)

    def prep(g, c):
        _relayout(wq_v, wq2_v, g, c, M // GROUP)
        _relayout(wuk_v, wuk2_v, g, c, Dc // GROUP)
        _relayout(wuv_v, wuv2_v, g, c, Dc // GROUP)

    for c in range(GROUP):
        prep(0, c)

    def pair(j, _):
        prep(jnp.minimum(j // GROUP + 1, NPAIRS // GROUP - 1), j % GROUP)
        q2 = jnp.dot(xn_v[...], wq2_v[j], preferred_element_type=F32) * qscale
        q_v[0] = q2[:, :D].astype(BF16)
        q_v[1] = q2[:, D:].astype(BF16)
        k2 = jnp.dot(ckv_v[...], wuk2_v[j], preferred_element_type=F32)
        k_v[0] = k2[:, :D].astype(BF16)
        k_v[1] = k2[:, D:].astype(BF16)
        v2 = jnp.dot(ckv_v[...], wuv2_v[j], preferred_element_type=F32)
        v_v[0] = v2[:, :D].astype(BF16)
        v_v[1] = v2[:, D:].astype(BF16)

        def head(e, _):
            attend(e, 2 * j + e)
            return 0
        lax.fori_loop(0, 2, head, 0)
        return 0
    lax.fori_loop(0, npairs, pair, 0)

    c_wo.wait()
    wr8 = jnp.broadcast_to(wr_ref[...], (8, M))

    def oproj(b, _):
        r0 = pl.multiple_of(b * RB, RB)
        rows = pl.ds(r0, RB)
        ctx = jnp.concatenate([ctx_v[h, rows, :] for h in range(H)], axis=1)
        a = jnp.dot(ctx, wo_v[...], preferred_element_type=F32)
        hh = (x_v[rows, :].astype(F32) + a).astype(BF16).astype(F32)
        hn = _layernorm(hh).astype(BF16)
        xn_v[rows, :] = hn
        out_ref[rows, :] = (hh + hn.astype(F32)).astype(BF16)
        r = lax.dot_general(wr8, hn, NT, preferred_element_type=F32)
        r_v[:, rows] = r.astype(BF16).astype(F32)
        return 0
    lax.fori_loop(0, S // RB, oproj, 0)

    r = r_v[0:1, :]
    pos = lax.broadcasted_iota(jnp.int32, (1, S), 1)
    m1 = jnp.max(r, axis=1, keepdims=True)
    i1 = jnp.min(jnp.where(r == m1, pos, S), axis=1, keepdims=True)
    r2 = jnp.where(pos == i1, -jnp.inf, r)
    m2 = jnp.max(r2, axis=1, keepdims=True)
    i2 = jnp.min(jnp.where(r2 == m2, pos, S), axis=1, keepdims=True)
    idx = [jnp.clip(jnp.min(i), 0, S - 1) for i in (i1, i2)]
    sub = lax.broadcasted_iota(jnp.int32, (16, M), 0)
    tiles = [pl.ds(pl.multiple_of((i // 16) * 16, 16), 16) for i in idx]
    sel = [sub == (i % 16) for i in idx]
    xs = [jnp.sum(jnp.where(s, xn_v[t, :].astype(F32), 0.0), axis=0, keepdims=True) for s, t in zip(sel, tiles)]
    x2 = jnp.where(sub == 0, xs[0], jnp.where(sub == 1, xs[1], 0.0)).astype(BF16)
    c_wg.wait(); c_wu.wait(); c_wd.wait()
    g = jnp.dot(x2, wg_v[...], preferred_element_type=F32)
    u = jnp.dot(x2, wu_v[...], preferred_element_type=F32)
    a = (g * jax.nn.sigmoid(g) * u).astype(BF16)
    y = jnp.dot(a, wd_v[...], preferred_element_type=F32)
    for n, mv in enumerate((m1, m2)):
        yn = y[n:n + 1, :] * jax.nn.sigmoid(mv)
        t = out_ref[tiles[n], :].astype(F32)
        out_ref[tiles[n], :] = jnp.where(sel[n], t + yn, t).astype(BF16)


@jax.jit
def pallas_sequential_preLN__compressed_kv_cla__moe_arch_mod__prompt_kernel(
    A_x, A_c_kv, A_w_q, A_w_uk, A_w_uv, A_w_o, B_x, B_w_r, B_w_gate, B_w_up, B_w_down,
):
    del B_x
    B, S, M = A_x.shape
    _, H, D = A_w_q.shape
    Dc = A_c_kv.shape[2]
    Fd = B_w_gate.shape[1]
    assert B == 1 and A_c_kv.shape[1] == S
    hbm = pl.BlockSpec(memory_space=pl.ANY)
    vm = lambda shape, dt=BF16: pltpu.VMEM(shape, dt)
    out = pl.pallas_call(
        functools.partial(_kernel, S=S, M=M, H=H, D=D, Dc=Dc),
        in_specs=[hbm] * 6 + [pl.BlockSpec(memory_space=pltpu.VMEM)] + [hbm] * 3,
        out_specs=pl.BlockSpec(memory_space=pltpu.VMEM),
        out_shape=jax.ShapeDtypeStruct((S, M), BF16),
        scratch_shapes=[
            vm((S, M)), vm((S, Dc)), vm((M * H, D)), vm((Dc * H, D)), vm((Dc * H, D)), vm((H * D, M)),
            vm((M, Fd)), vm((M, Fd)), vm((Fd, M)),
            vm((H // 2, M, 2 * D)), vm((H // 2, Dc, 2 * D)), vm((H // 2, Dc, 2 * D)),
            vm((S, M)), vm((2, S, D)), vm((2, S, D)), vm((2, S, D)), vm((H, S, D)), vm((8, S), F32),
            pltpu.SemaphoreType.DMA((9,)),
        ],
        compiler_params=pltpu.CompilerParams(vmem_limit_bytes=120 * 1024 * 1024),
    )(
        A_x.reshape(S, M), A_c_kv.reshape(S, Dc), A_w_q.reshape(M * H, D), A_w_uk.reshape(Dc * H, D),
        A_w_uv.reshape(Dc * H, D), A_w_o.reshape(H * D, M), B_w_r.reshape(1, M), B_w_gate, B_w_up, B_w_down,
    )
    return out.reshape(B, S, M)
```

```python
import contextlib
import functools
import math

import jax
import jax.numpy as jnp
from jax import lax
import jax.experimental.pallas as pl
import jax.experimental.pallas.tpu as pltpu

F32 = jnp.float32
BF16 = jnp.bfloat16
EPS = 1e-5
BQ = 512
BK = 2048
SAFE = 32.0
OB = 512
RB = 256
NPAIRS = 16
GROUP = 4
NT = (((1,), (1,)), ((), ()))


PROFILE = False


def _scope(name):
    return jax.named_scope(name) if PROFILE else contextlib.nullcontext()


def _fold(x, op):
    r = x[:, :128]
    for c in range(128, x.shape[1], 128):
        r = op(r, x[:, c:c + 128])
    return r


def _recip(x):
    r = pl.reciprocal(x, approx=True)
    return r * (2.0 - x * r)


def _max_sq_norm(x):
    n = jnp.sum(x * x, axis=1, keepdims=True)
    return jnp.max(n)


def _layernorm(x):
    m = jnp.mean(x, axis=-1, keepdims=True)
    d = x - m
    v = jnp.mean(d * d, axis=-1, keepdims=True)
    return d * lax.rsqrt(v + EPS)


def _relayout(w_ref, dst_ref, g, c, rows):
    m0 = pl.multiple_of(c * rows, rows)
    base = pl.multiple_of(m0 * NPAIRS + g * GROUP, GROUP)
    win = w_ref.bitcast(jnp.uint32).at[pl.ds(base, (rows - 1) * NPAIRS + GROUP), :]
    for s in range(GROUP):
        u = win[pl.ds(s, rows, stride=NPAIRS), :]
        lo = pltpu.bitcast(u << 16, F32).astype(BF16)
        hi = pltpu.bitcast(u & jnp.uint32(0xFFFF0000), F32).astype(BF16)
        dst_ref[g * GROUP + s, pl.ds(m0, rows), :] = jnp.concatenate([lo, hi], axis=1)


def _kernel(x_hbm, ckv_hbm, wq_hbm, wuk_hbm, wuv_hbm, wo_hbm, wr_ref, wg_hbm, wu_hbm, wd_hbm, out_hbm,
            x_v, ckv_v, wq_v, wuk_v, wuv_v, wo_v, wg_v, wu_v, wd_v,
            wq2_v, wuk2_v, wuv2_v, xn_v, q_v, k_v, v_v, r_v, out_ref, sems, *, S, M, H, D, Dc):
    npairs = H // 2
    cp = lambda i, s, d: pltpu.make_async_copy(s, d, sems.at[i])
    c_x, c_ckv, c_wq = cp(0, x_hbm, x_v), cp(1, ckv_hbm, ckv_v), cp(2, wq_hbm, wq_v)
    c_wuk, c_wuv, c_wo = cp(3, wuk_hbm, wuk_v), cp(4, wuv_hbm, wuv_v), cp(5, wo_hbm, wo_v)
    c_wg, c_wu, c_wd = cp(6, wg_hbm, wg_v), cp(7, wu_hbm, wu_v), cp(8, wd_hbm, wd_v)
    def prep_v(g, c):
        _relayout(wuv_v, wuv2_v, g, c, Dc // GROUP)

    def prep_qk(g, c):
        _relayout(wq_v, wq2_v, g, c, M // GROUP)
        _relayout(wuk_v, wuk2_v, g, c, Dc // GROUP)

    def next_group(j):
        return jnp.minimum(j // GROUP + 1, NPAIRS // GROUP - 1)

    c_ckv.start(); c_wuv.start()
    with _scope('wait_first'):
        c_ckv.wait(); c_wuv.wait()
    for c in (c_x, c_wq, c_wuk):
        c.start()
    for c in range(GROUP):
        prep_v(0, c)

    def vproj(j, _):
        prep_v(next_group(j), j % GROUP)
        v2 = jnp.dot(ckv_v[...], wuv2_v[j], preferred_element_type=F32)
        v_v[2 * j + 1] = v2[:, :D].astype(BF16)
        v_v[2 * j + 2] = v2[:, D:].astype(BF16)
        return 0

    def vproj_ln(j, _):
        vproj(j, 0)
        b = j - (NPAIRS - S // RB)
        rows = pl.ds(pl.multiple_of(b * RB, RB), RB)
        xn_v[rows, :] = _layernorm(x_v[rows, :].astype(F32)).astype(BF16)
        prep_qk(0, j % GROUP)
        return 0

    with _scope('vproj1'):
        lax.fori_loop(0, NPAIRS - S // RB, vproj, 0)
    with _scope('wait_x'):
        c_x.wait(); c_wq.wait(); c_wuk.wait()
    for c in (c_wo, c_wg, c_wu, c_wd):
        c.start()
    with _scope('vproj2'):
        lax.fori_loop(NPAIRS - S // RB, NPAIRS, vproj_ln, 0)

    qscale = (D ** -0.5) * math.log2(math.e)
    nq = S // BQ

    def attend(e, h, shift):
        T = 128
        tri = (lax.broadcasted_iota(jnp.int32, (T, T), 1) <= lax.broadcasted_iota(jnp.int32, (T, T), 0))
        nt = BQ // T
        for i in range(nq):
            r0 = i * BQ
            q = q_v[e, r0:r0 + BQ, :]
            pieces = []
            for c0 in range(0, r0, BK):
                c1 = min(c0 + BK, r0)
                pieces.append((0, c0, c1, lax.dot_general(q, k_v[e, c0:c1, :], NT, preferred_element_type=F32)))
            for t in range(nt):
                c0 = r0 + t * T
                sd = lax.dot_general(q[t * T:], k_v[e, c0:c0 + T, :], NT, preferred_element_type=F32)
                top = jnp.where(tri, sd[:T], -1e9)
                sd = top if t == nt - 1 else jnp.concatenate([top, sd[T:]], axis=0)
                pieces.append((t, c0, c0 + T, sd))
            rowtile = lambda a, t0, u: a[(u - t0) * T:(u - t0 + 1) * T]
            if shift:
                m = []
                for u in range(nt):
                    mu = None
                    for t0, _, _, sc in pieces:
                        if t0 <= u:
                            x = jnp.max(_fold(rowtile(sc, t0, u), jnp.maximum), axis=1, keepdims=True)
                            mu = x if mu is None else jnp.maximum(mu, x)
                    m.append(mu)
            o = [None] * nt
            l = [None] * nt
            for t0, c0, c1, sc in pieces:
                if shift:
                    sc = sc - jnp.concatenate(m[t0:], axis=0)
                p = jnp.exp2(sc)
                pv = jnp.dot(p.astype(BF16), v_v[h + 1, c0:c1, :], preferred_element_type=F32)
                ps = _fold(p, jnp.add)
                for u in range(t0, nt):
                    a, b = rowtile(pv, t0, u), rowtile(ps, t0, u)
                    o[u] = a if o[u] is None else o[u] + a
                    l[u] = b if l[u] is None else l[u] + b
            for u in range(nt):
                ls = jnp.sum(l[u], axis=1, keepdims=True)
                v_v[h, r0 + u * T:r0 + (u + 1) * T, :] = (o[u] * _recip(ls)).astype(BF16)

    def pair(j, _):
        prep_qk(next_group(j), j % GROUP)
        q2 = jnp.dot(xn_v[...], wq2_v[j], preferred_element_type=F32) * qscale
        q_v[0] = q2[:, :D].astype(BF16)
        q_v[1] = q2[:, D:].astype(BF16)
        k2 = jnp.dot(ckv_v[...], wuk2_v[j], preferred_element_type=F32)
        k_v[0] = k2[:, :D].astype(BF16)
        k_v[1] = k2[:, D:].astype(BF16)
        safe = [_max_sq_norm(q2[:, n * D:(n + 1) * D]) * _max_sq_norm(k2[:, n * D:(n + 1) * D]) <= SAFE * SAFE
                for n in range(2)]

        def head(e, _):
            ok = jnp.where(e == 0, safe[0], safe[1])
            pl.when(ok)(lambda: attend(e, 2 * j + e, False))
            pl.when(jnp.logical_not(ok))(lambda: attend(e, 2 * j + e, True))
            return 0
        with _scope('attn'):
            lax.fori_loop(0, 2, head, 0)
        return 0
    with _scope('pairs'):
        lax.fori_loop(0, npairs, pair, 0)

    c_wo.wait()
    wr8 = jnp.broadcast_to(wr_ref[...], (8, M))

    def out_copy(rows, sem=9):
        return pltpu.make_async_copy(out_ref.at[rows], out_hbm.at[rows], sems.at[sem])

    def oproj(b, _):
        r0 = pl.multiple_of(b * OB, OB)
        rows = pl.ds(r0, OB)
        ctx = jnp.concatenate([v_v[h, rows, :] for h in range(H)], axis=1)
        a = jnp.dot(ctx, wo_v[...], preferred_element_type=F32)
        hh = (x_v[rows, :].astype(F32) + a).astype(BF16).astype(F32)
        hn = _layernorm(hh).astype(BF16)
        xn_v[rows, :] = hn
        out_ref[rows, :] = (hh + hn.astype(F32)).astype(BF16)
        r = lax.dot_general(wr8, hn, NT, preferred_element_type=F32)
        r_v[:, rows] = r.astype(BF16).astype(F32)
        out_copy(rows).start()
        return 0
    with _scope('oproj'):
        lax.fori_loop(0, S // OB, oproj, 0)

    r = r_v[0:1, :]
    pos = lax.broadcasted_iota(jnp.int32, (1, S), 1)
    m1 = jnp.max(r, axis=1, keepdims=True)
    i1 = jnp.min(jnp.where(r == m1, pos, S), axis=1, keepdims=True)
    r2 = jnp.where(pos == i1, -jnp.inf, r)
    m2 = jnp.max(r2, axis=1, keepdims=True)
    i2 = jnp.min(jnp.where(r2 == m2, pos, S), axis=1, keepdims=True)
    idx = [jnp.clip(jnp.min(i), 0, S - 1) for i in (i1, i2)]
    sub = lax.broadcasted_iota(jnp.int32, (16, M), 0)
    tiles = [pl.ds(pl.multiple_of((i // 16) * 16, 16), 16) for i in idx]
    sel = [sub == (i % 16) for i in idx]
    xs = [jnp.sum(jnp.where(s, xn_v[t, :].astype(F32), 0.0), axis=0, keepdims=True) for s, t in zip(sel, tiles)]
    x2 = jnp.where(sub == 0, xs[0], jnp.where(sub == 1, xs[1], 0.0)).astype(BF16)
    c_wg.wait(); c_wu.wait(); c_wd.wait()
    g = jnp.dot(x2, wg_v[...], preferred_element_type=F32)
    u = jnp.dot(x2, wu_v[...], preferred_element_type=F32)
    a = (g * jax.nn.sigmoid(g) * u).astype(BF16)
    y = jnp.dot(a, wd_v[...], preferred_element_type=F32)
    out_copy(slice(None)).wait()
    for n, mv in enumerate((m1, m2)):
        yn = y[n:n + 1, :] * jax.nn.sigmoid(mv)
        t = out_ref[tiles[n], :].astype(F32)
        out_ref[tiles[n], :] = jnp.where(sel[n], t + yn, t).astype(BF16)
    out_copy(tiles[0], 9).start()

    @pl.when(idx[0] // 16 != idx[1] // 16)
    def _():
        out_copy(tiles[1], 10).start()
        out_copy(tiles[1], 10).wait()
    out_copy(tiles[0], 9).wait()


@jax.jit
def pallas_sequential_preLN__compressed_kv_cla__moe_arch_mod__prompt_kernel(
    A_x, A_c_kv, A_w_q, A_w_uk, A_w_uv, A_w_o, B_x, B_w_r, B_w_gate, B_w_up, B_w_down,
):
    del B_x
    B, S, M = A_x.shape
    _, H, D = A_w_q.shape
    Dc = A_c_kv.shape[2]
    Fd = B_w_gate.shape[1]
    assert B == 1 and A_c_kv.shape[1] == S
    hbm = pl.BlockSpec(memory_space=pl.ANY)
    vm = lambda shape, dt=BF16: pltpu.VMEM(shape, dt)
    out = pl.pallas_call(
        functools.partial(_kernel, S=S, M=M, H=H, D=D, Dc=Dc),
        in_specs=[hbm] * 6 + [pl.BlockSpec(memory_space=pltpu.VMEM)] + [hbm] * 3,
        out_specs=hbm,
        out_shape=jax.ShapeDtypeStruct((S, M), BF16),
        scratch_shapes=[
            vm((S, M)), vm((S, Dc)), vm((M * H, D)), vm((Dc * H, D)), vm((Dc * H, D)), vm((H * D, M)),
            vm((M, Fd)), vm((M, Fd)), vm((Fd, M)),
            vm((H // 2, M, 2 * D)), vm((H // 2, Dc, 2 * D)), vm((H // 2, Dc, 2 * D)),
            vm((S, M)), vm((2, S, D)), vm((2, S, D)), vm((H + 1, S, D)), vm((8, S), F32), vm((S, M)),
            pltpu.SemaphoreType.DMA((11,)),
        ],
        compiler_params=pltpu.CompilerParams(vmem_limit_bytes=120 * 1024 * 1024),
    )(
        A_x.reshape(S, M), A_c_kv.reshape(S, Dc), A_w_q.reshape(M * H, D), A_w_uk.reshape(Dc * H, D),
        A_w_uv.reshape(Dc * H, D), A_w_o.reshape(H * D, M), B_w_r.reshape(1, M), B_w_gate, B_w_up, B_w_down,
    )
    return out.reshape(B, S, M)
```

```python
import contextlib
import functools
import math

import jax
import jax.numpy as jnp
from jax import lax
import jax.experimental.pallas as pl
import jax.experimental.pallas.tpu as pltpu

F32 = jnp.float32
BF16 = jnp.bfloat16
EPS = 1e-5
BQ = 512
BK = 2048
SAFE = 32.0
OB = 512
RB = 256
NPAIRS = 16
GROUP = 4
NT = (((1,), (1,)), ((), ()))


PROFILE = False


def _scope(name):
    return jax.named_scope(name) if PROFILE else contextlib.nullcontext()


def _fold(x, op):
    r = x[:, :128]
    for c in range(128, x.shape[1], 128):
        r = op(r, x[:, c:c + 128])
    return r


def _recip(x):
    r = pl.reciprocal(x, approx=True)
    return r * (2.0 - x * r)


def _max_sq_norm(x):
    n = jnp.sum(x * x, axis=1, keepdims=True)
    return jnp.max(n)


def _layernorm(x):
    m = jnp.mean(x, axis=-1, keepdims=True)
    d = x - m
    v = jnp.mean(d * d, axis=-1, keepdims=True)
    return d * lax.rsqrt(v + EPS)


def _relayout(w_ref, dst_ref, g, c, rows):
    m0 = pl.multiple_of(c * rows, rows)
    base = pl.multiple_of(m0 * NPAIRS + g * GROUP, GROUP)
    win = w_ref.bitcast(jnp.uint32).at[pl.ds(base, (rows - 1) * NPAIRS + GROUP), :]
    for s in range(GROUP):
        u = win[pl.ds(s, rows, stride=NPAIRS), :]
        lo = pltpu.bitcast(u << 16, F32).astype(BF16)
        hi = pltpu.bitcast(u & jnp.uint32(0xFFFF0000), F32).astype(BF16)
        dst_ref[g * GROUP + s, pl.ds(m0, rows), :] = jnp.concatenate([lo, hi], axis=1)


def _kernel(x_hbm, ckv_hbm, wq_hbm, wuk_hbm, wuv_hbm, wo_hbm, wr_ref, wg_hbm, wu_hbm, wd_hbm, out_hbm,
            x_v, ckv_v, wq_v, wuk_v, wuv_v, wo_v, wg_v, wu_v, wd_v,
            wq2_v, wuk2_v, wuv2_v, xn_v, q_v, k_v, v_v, r_v, out_ref, ok_s, sems, *, S, M, H, D, Dc):
    npairs = H // 2
    cp = lambda i, s, d: pltpu.make_async_copy(s, d, sems.at[i])
    c_x, c_ckv, c_wq = cp(0, x_hbm, x_v), cp(1, ckv_hbm, ckv_v), cp(2, wq_hbm, wq_v)
    c_wuk, c_wuv, c_wo = cp(3, wuk_hbm, wuk_v), cp(4, wuv_hbm, wuv_v), cp(5, wo_hbm, wo_v)
    c_wg, c_wu, c_wd = cp(6, wg_hbm, wg_v), cp(7, wu_hbm, wu_v), cp(8, wd_hbm, wd_v)
    def prep_v(g, c):
        _relayout(wuv_v, wuv2_v, g, c, Dc // GROUP)

    def prep_qk(g, c):
        _relayout(wq_v, wq2_v, g, c, M // GROUP)
        _relayout(wuk_v, wuk2_v, g, c, Dc // GROUP)

    def next_group(j):
        return jnp.minimum(j // GROUP + 1, NPAIRS // GROUP - 1)

    c_ckv.start(); c_wuv.start()
    with _scope('wait_first'):
        c_ckv.wait(); c_wuv.wait()
    for c in (c_x, c_wq, c_wuk):
        c.start()
    for c in range(GROUP):
        prep_v(0, c)

    def vproj(j, _):
        prep_v(next_group(j), j % GROUP)
        v2 = jnp.dot(ckv_v[...], wuv2_v[j], preferred_element_type=F32)
        v_v[2 * j + 1] = v2[:, :D].astype(BF16)
        v_v[2 * j + 2] = v2[:, D:].astype(BF16)
        return 0

    def vproj_ln(j, _):
        vproj(j, 0)
        b = j - (NPAIRS - S // RB)
        rows = pl.ds(pl.multiple_of(b * RB, RB), RB)
        xn_v[rows, :] = _layernorm(x_v[rows, :].astype(F32)).astype(BF16)
        prep_qk(0, j % GROUP)
        return 0

    with _scope('vproj1'):
        lax.fori_loop(0, NPAIRS - S // RB, vproj, 0, unroll=True)
    with _scope('wait_x'):
        c_x.wait(); c_wq.wait(); c_wuk.wait()
    for c in (c_wo, c_wg, c_wu, c_wd):
        c.start()
    with _scope('vproj2'):
        lax.fori_loop(NPAIRS - S // RB, NPAIRS, vproj_ln, 0, unroll=True)

    qscale = (D ** -0.5) * math.log2(math.e)
    nq = S // BQ

    def attend(e, h, shift):
        T = 128
        tri = (lax.broadcasted_iota(jnp.int32, (T, T), 1) <= lax.broadcasted_iota(jnp.int32, (T, T), 0))
        nt = BQ // T
        for i in range(nq):
            r0 = i * BQ
            q = q_v[e, r0:r0 + BQ, :]
            pieces = []
            for c0 in range(0, r0, BK):
                c1 = min(c0 + BK, r0)
                pieces.append((0, c0, c1, lax.dot_general(q, k_v[e, c0:c1, :], NT, preferred_element_type=F32)))
            for t in range(nt):
                c0 = r0 + t * T
                sd = lax.dot_general(q[t * T:], k_v[e, c0:c0 + T, :], NT, preferred_element_type=F32)
                top = jnp.where(tri, sd[:T], -1e9)
                sd = top if t == nt - 1 else jnp.concatenate([top, sd[T:]], axis=0)
                pieces.append((t, c0, c0 + T, sd))
            rowtile = lambda a, t0, u: a[(u - t0) * T:(u - t0 + 1) * T]
            if shift:
                m = []
                for u in range(nt):
                    mu = None
                    for t0, _, _, sc in pieces:
                        if t0 <= u:
                            x = jnp.max(_fold(rowtile(sc, t0, u), jnp.maximum), axis=1, keepdims=True)
                            mu = x if mu is None else jnp.maximum(mu, x)
                    m.append(mu)
            o = [None] * nt
            l = [None] * nt
            for t0, c0, c1, sc in pieces:
                if shift:
                    sc = sc - jnp.concatenate(m[t0:], axis=0)
                p = jnp.exp2(sc)
                pv = jnp.dot(p.astype(BF16), v_v[h + 1, c0:c1, :], preferred_element_type=F32)
                ps = _fold(p, jnp.add)
                for u in range(t0, nt):
                    a, b = rowtile(pv, t0, u), rowtile(ps, t0, u)
                    o[u] = a if o[u] is None else o[u] + a
                    l[u] = b if l[u] is None else l[u] + b
            for u in range(nt):
                ls = jnp.sum(l[u], axis=1, keepdims=True)
                v_v[h, r0 + u * T:r0 + (u + 1) * T, :] = (o[u] * _recip(ls)).astype(BF16)

    def qkproj(j):
        slot = 2 * (j % 2)
        prep_qk(next_group(j), j % GROUP)
        q2 = jnp.dot(xn_v[...], wq2_v[j], preferred_element_type=F32) * qscale
        q_v[slot] = q2[:, :D].astype(BF16)
        q_v[slot + 1] = q2[:, D:].astype(BF16)
        k2 = jnp.dot(ckv_v[...], wuk2_v[j], preferred_element_type=F32)
        k_v[slot] = k2[:, :D].astype(BF16)
        k_v[slot + 1] = k2[:, D:].astype(BF16)
        bound = [_max_sq_norm(q2[:, n * D:(n + 1) * D]) * _max_sq_norm(k2[:, n * D:(n + 1) * D])
                 for n in range(2)]
        ok_s[j % 2] = (jnp.maximum(bound[0], bound[1]) <= SAFE * SAFE).astype(jnp.int32)

    qkproj(0)

    def pair(j, _):
        pl.when(j + 1 < NPAIRS)(lambda: qkproj(j + 1))
        slot = 2 * (j % 2)
        ok = ok_s[j % 2] == 1

        @pl.when(ok)
        def _():
            with _scope('attn'):
                lax.fori_loop(0, 2, lambda e, c: attend(slot + e, 2 * j + e, False) or 0, 0)

        @pl.when(jnp.logical_not(ok))
        def _():
            def head(e, _):
                attend(slot + e, 2 * j + e, True)
                return 0
            lax.fori_loop(0, 2, head, 0)
        return 0
    with _scope('pairs'):
        lax.fori_loop(0, npairs, pair, 0)

    c_wo.wait()
    wr8 = jnp.broadcast_to(wr_ref[...], (8, M))

    def out_copy(rows, sem=9):
        return pltpu.make_async_copy(out_ref.at[rows], out_hbm.at[rows], sems.at[sem])

    def oproj(b, _):
        r0 = pl.multiple_of(b * OB, OB)
        rows = pl.ds(r0, OB)
        ctx = jnp.concatenate([v_v[h, rows, :] for h in range(H)], axis=1)
        a = jnp.dot(ctx, wo_v[...], preferred_element_type=F32)
        hh = (x_v[rows, :].astype(F32) + a).astype(BF16).astype(F32)
        hn = _layernorm(hh).astype(BF16)
        xn_v[rows, :] = hn
        out_ref[rows, :] = (hh + hn.astype(F32)).astype(BF16)
        r = lax.dot_general(wr8, hn, NT, preferred_element_type=F32)
        r_v[:, rows] = r.astype(BF16).astype(F32)
        out_copy(rows).start()
        return 0
    with _scope('oproj'):
        lax.fori_loop(0, S // OB, oproj, 0)

    r = r_v[0:1, :]
    pos = lax.broadcasted_iota(jnp.int32, (1, S), 1)
    m1 = jnp.max(r, axis=1, keepdims=True)
    i1 = jnp.min(jnp.where(r == m1, pos, S), axis=1, keepdims=True)
    r2 = jnp.where(pos == i1, -jnp.inf, r)
    m2 = jnp.max(r2, axis=1, keepdims=True)
    i2 = jnp.min(jnp.where(r2 == m2, pos, S), axis=1, keepdims=True)
    idx = [jnp.clip(jnp.min(i), 0, S - 1) for i in (i1, i2)]
    sub = lax.broadcasted_iota(jnp.int32, (16, M), 0)
    tiles = [pl.ds(pl.multiple_of((i // 16) * 16, 16), 16) for i in idx]
    sel = [sub == (i % 16) for i in idx]
    xs = [jnp.sum(jnp.where(s, xn_v[t, :].astype(F32), 0.0), axis=0, keepdims=True) for s, t in zip(sel, tiles)]
    x2 = jnp.where(sub == 0, xs[0], jnp.where(sub == 1, xs[1], 0.0)).astype(BF16)
    c_wg.wait(); c_wu.wait(); c_wd.wait()
    g = jnp.dot(x2, wg_v[...], preferred_element_type=F32)
    u = jnp.dot(x2, wu_v[...], preferred_element_type=F32)
    a = (g * jax.nn.sigmoid(g) * u).astype(BF16)
    y = jnp.dot(a, wd_v[...], preferred_element_type=F32)
    out_copy(slice(None)).wait()
    for n, mv in enumerate((m1, m2)):
        yn = y[n:n + 1, :] * jax.nn.sigmoid(mv)
        t = out_ref[tiles[n], :].astype(F32)
        out_ref[tiles[n], :] = jnp.where(sel[n], t + yn, t).astype(BF16)
    out_copy(tiles[0], 9).start()

    @pl.when(idx[0] // 16 != idx[1] // 16)
    def _():
        out_copy(tiles[1], 10).start()
        out_copy(tiles[1], 10).wait()
    out_copy(tiles[0], 9).wait()


@jax.jit
def pallas_sequential_preLN__compressed_kv_cla__moe_arch_mod__prompt_kernel(
    A_x, A_c_kv, A_w_q, A_w_uk, A_w_uv, A_w_o, B_x, B_w_r, B_w_gate, B_w_up, B_w_down,
):
    del B_x
    B, S, M = A_x.shape
    _, H, D = A_w_q.shape
    Dc = A_c_kv.shape[2]
    Fd = B_w_gate.shape[1]
    assert B == 1 and A_c_kv.shape[1] == S
    hbm = pl.BlockSpec(memory_space=pl.ANY)
    vm = lambda shape, dt=BF16: pltpu.VMEM(shape, dt)
    out = pl.pallas_call(
        functools.partial(_kernel, S=S, M=M, H=H, D=D, Dc=Dc),
        in_specs=[hbm] * 6 + [pl.BlockSpec(memory_space=pltpu.VMEM)] + [hbm] * 3,
        out_specs=hbm,
        out_shape=jax.ShapeDtypeStruct((S, M), BF16),
        scratch_shapes=[
            vm((S, M)), vm((S, Dc)), vm((M * H, D)), vm((Dc * H, D)), vm((Dc * H, D)), vm((H * D, M)),
            vm((M, Fd)), vm((M, Fd)), vm((Fd, M)),
            vm((H // 2, M, 2 * D)), vm((H // 2, Dc, 2 * D)), vm((H // 2, Dc, 2 * D)),
            vm((S, M)), vm((4, S, D)), vm((4, S, D)), vm((H + 1, S, D)), vm((8, S), F32), vm((S, M)),
            pltpu.SMEM((2,), jnp.int32),
            pltpu.SemaphoreType.DMA((11,)),
        ],
        compiler_params=pltpu.CompilerParams(vmem_limit_bytes=120 * 1024 * 1024),
    )(
        A_x.reshape(S, M), A_c_kv.reshape(S, Dc), A_w_q.reshape(M * H, D), A_w_uk.reshape(Dc * H, D),
        A_w_uv.reshape(Dc * H, D), A_w_o.reshape(H * D, M), B_w_r.reshape(1, M), B_w_gate, B_w_up, B_w_down,
    )
    return out.reshape(B, S, M)
```

```python
import contextlib
import functools
import math

import jax
import jax.numpy as jnp
from jax import lax
import jax.experimental.pallas as pl
import jax.experimental.pallas.tpu as pltpu

F32 = jnp.float32
BF16 = jnp.bfloat16
EPS = 1e-5
BQ = 2048
BK = 2048
SAFE = 32.0
OB = 512
AHEAD = 4
RB = 256
NPAIRS = 16
NT = (((1,), (1,)), ((), ()))


PROFILE = False


def _scope(name):
    return jax.named_scope(name) if PROFILE else contextlib.nullcontext()


def _fold(x, op):
    r = x[:, :128]
    for c in range(128, x.shape[1], 128):
        r = op(r, x[:, c:c + 128])
    return r


def _recip(x):
    r = pl.reciprocal(x, approx=True)
    return r * (2.0 - x * r)


def _max_sq_norm(x):
    n = jnp.sum(x * x, axis=1, keepdims=True)
    return jnp.max(n)


def _layernorm(x):
    m = jnp.mean(x, axis=-1, keepdims=True)
    d = x - m
    v = jnp.mean(d * d, axis=-1, keepdims=True)
    return d * lax.rsqrt(v + EPS)


def _pair_copies(w_hbm, buf, sems, j):
    w32 = w_hbm.bitcast(jnp.uint32)
    return [pltpu.make_async_copy(w32.at[:, j + e * NPAIRS, :], buf.at[j, e], sems.at[j]) for e in range(2)]


def _pair_weights(buf, j):
    ev, od = buf[j, 0], buf[j, 1]
    lo = (ev & jnp.uint32(0xFFFF)) | (od << 16)
    hi = (ev >> 16) | (od & jnp.uint32(0xFFFF0000))
    return jnp.concatenate([pltpu.bitcast(lo, BF16), pltpu.bitcast(hi, BF16)], axis=1)


def _kernel(x_hbm, ckv_hbm, wq_hbm, wuk_hbm, wuv_hbm, wo_hbm, wr_ref, wg_hbm, wu_hbm, wd_hbm, out_hbm,
            x_v, ckv_v, wq_v, wuk_v, wuv_v, wo_v, wg_v, wu_v, wd_v,
            xn_v, q_v, k_v, v_v, r_v, out_ref, ok_s, sems, qsem, ksem, vsem, *, S, M, H, D, Dc):
    npairs = H // 2
    cp = lambda i, s, d: pltpu.make_async_copy(s, d, sems.at[i])
    c_x, c_ckv, c_wo = cp(0, x_hbm, x_v), cp(1, ckv_hbm, ckv_v), cp(5, wo_hbm, wo_v)
    q_copies = lambda j: _pair_copies(wq_hbm, wq_v, qsem, j)
    k_copies = lambda j: _pair_copies(wuk_hbm, wuk_v, ksem, j)
    v_copies = lambda j: _pair_copies(wuv_hbm, wuv_v, vsem, j)

    def start(copies):
        for c in copies:
            c.start()

    def wait(copies):
        for c in copies:
            c.wait()
    c_wg, c_wu, c_wd = cp(6, wg_hbm, wg_v), cp(7, wu_hbm, wu_v), cp(8, wd_hbm, wd_v)
    c_ckv.start()
    for j in range(AHEAD):
        start(v_copies(j))
    with _scope('wait_first'):
        c_ckv.wait()
    c_x.start()

    def vproj(j, _):
        if j + AHEAD < NPAIRS:
            start(v_copies(j + AHEAD))
        start(q_copies(j) + k_copies(j))
        wait(v_copies(j))
        v2 = jnp.dot(ckv_v[...], _pair_weights(wuv_v, j), preferred_element_type=F32)
        v_v[2 * j + 1] = v2[:, :D].astype(BF16)
        v_v[2 * j + 2] = v2[:, D:].astype(BF16)
        return 0

    def vproj_ln(j, _):
        vproj(j, 0)
        b = j - (NPAIRS - S // RB)
        rows = pl.ds(b * RB, RB)
        xn_v[rows, :] = _layernorm(x_v[rows, :].astype(F32)).astype(BF16)
        return 0

    with _scope('vproj1'):
        for j in range(NPAIRS - S // RB):
            vproj(j, 0)
    with _scope('wait_x'):
        c_x.wait()
    with _scope('vproj2'):
        for j in range(NPAIRS - S // RB, NPAIRS):
            vproj_ln(j, 0)

    qscale = (D ** -0.5) * math.log2(math.e)
    nq = S // BQ

    def attend(e, h):
        T = 128
        tri = (lax.broadcasted_iota(jnp.int32, (T, T), 1) <= lax.broadcasted_iota(jnp.int32, (T, T), 0))
        nt = BQ // T
        for i in range(nq):
            r0 = i * BQ
            q = q_v[e, r0:r0 + BQ, :]
            pieces = []
            for c0 in range(0, r0, BK):
                c1 = min(c0 + BK, r0)
                pieces.append((0, c0, c1, lax.dot_general(q, k_v[e, c0:c1, :], NT, preferred_element_type=F32)))
            for t in range(nt):
                c0 = r0 + t * T
                sd = lax.dot_general(q[t * T:], k_v[e, c0:c0 + T, :], NT, preferred_element_type=F32)
                top = jnp.where(tri, sd[:T], -1e9)
                sd = top if t == nt - 1 else jnp.concatenate([top, sd[T:]], axis=0)
                pieces.append((t, c0, c0 + T, sd))
            rowtile = lambda a, t0, u: a[(u - t0) * T:(u - t0 + 1) * T]
            o = [None] * nt
            l = [None] * nt
            for t0, c0, c1, sc in pieces:
                p = jnp.exp2(sc)
                pv = jnp.dot(p.astype(BF16), v_v[h + 1, c0:c1, :], preferred_element_type=F32)
                ps = _fold(p, jnp.add)
                for u in range(t0, nt):
                    a, b = rowtile(pv, t0, u), rowtile(ps, t0, u)
                    o[u] = a if o[u] is None else o[u] + a
                    l[u] = b if l[u] is None else l[u] + b
            for u in range(nt):
                ls = jnp.sum(l[u], axis=1, keepdims=True)
                v_v[h, r0 + u * T:r0 + (u + 1) * T, :] = (o[u] * _recip(ls)).astype(BF16)

    def attend_shifted(e, h):
        T = 256
        ri = lax.broadcasted_iota(jnp.int32, (T, T), 0)
        ci = lax.broadcasted_iota(jnp.int32, (T, T), 1)

        def qblock(i, _):
            rows = pl.ds(pl.multiple_of(i * T, T), T)
            q = q_v[e, rows, :]

            def kblock(c, carry):
                m, l, o = carry
                cols = pl.ds(pl.multiple_of(c * T, T), T)
                sc = lax.dot_general(q, k_v[e, cols, :], NT, preferred_element_type=F32)
                sc = jnp.where(ci + c * T <= ri + i * T, sc, -1e9)
                m_new = jnp.maximum(m, jnp.max(sc, axis=1, keepdims=True))
                alpha = jnp.exp2(m - m_new)
                p = jnp.exp2(sc - m_new)
                l = alpha * l + jnp.sum(p, axis=1, keepdims=True)
                o = alpha * o + jnp.dot(p.astype(BF16), v_v[h + 1, cols, :], preferred_element_type=F32)
                return m_new, l, o
            init = (jnp.full((T, 1), -jnp.inf, F32), jnp.zeros((T, 1), F32), jnp.zeros((T, D), F32))
            _, l, o = lax.fori_loop(0, i + 1, kblock, init)
            v_v[h, rows, :] = (o / l).astype(BF16)
            return 0
        lax.fori_loop(0, S // T, qblock, 0)

    def qkproj(j):
        slot = 2 * (j % 2)
        wait(q_copies(j) + k_copies(j))
        q2 = jnp.dot(xn_v[...], _pair_weights(wq_v, j), preferred_element_type=F32) * qscale
        q_v[slot] = q2[:, :D].astype(BF16)
        q_v[slot + 1] = q2[:, D:].astype(BF16)
        k2 = jnp.dot(ckv_v[...], _pair_weights(wuk_v, j), preferred_element_type=F32)
        k_v[slot] = k2[:, :D].astype(BF16)
        k_v[slot + 1] = k2[:, D:].astype(BF16)
        bound = [_max_sq_norm(q2[:, n * D:(n + 1) * D]) * _max_sq_norm(k2[:, n * D:(n + 1) * D])
                 for n in range(2)]
        ok_s[j % 2] = (jnp.maximum(bound[0], bound[1]) <= SAFE * SAFE).astype(jnp.int32)

    qkproj(0)

    def pair(j, _):
        @pl.when(j == 2)
        def _():
            for c in (c_wo, c_wg, c_wu, c_wd):
                c.start()
        pl.when(j + 1 < NPAIRS)(lambda: qkproj(j + 1))
        slot = 2 * (j % 2)
        ok = ok_s[j % 2] == 1

        @pl.when(ok)
        def _():
            with _scope('attn'):
                lax.fori_loop(0, 2, lambda e, c: attend(slot + e, 2 * j + e) or 0, 0)

        @pl.when(jnp.logical_not(ok))
        def _():
            def head(e, _):
                attend_shifted(slot + e, 2 * j + e)
                return 0
            lax.fori_loop(0, 2, head, 0)
        return 0
    with _scope('pairs'):
        lax.fori_loop(0, npairs, pair, 0)

    c_wo.wait()
    wr8 = jnp.broadcast_to(wr_ref[...], (8, M))

    def out_copy(rows, sem=9):
        return pltpu.make_async_copy(out_ref.at[rows], out_hbm.at[rows], sems.at[sem])

    def oproj(b, _):
        r0 = pl.multiple_of(b * OB, OB)
        rows = pl.ds(r0, OB)
        ctx = jnp.concatenate([v_v[h, rows, :] for h in range(H)], axis=1)
        a = jnp.dot(ctx, wo_v[...], preferred_element_type=F32)
        hh = (x_v[rows, :].astype(F32) + a).astype(BF16).astype(F32)
        hn = _layernorm(hh).astype(BF16)
        xn_v[rows, :] = hn
        out_ref[rows, :] = (hh + hn.astype(F32)).astype(BF16)
        r = lax.dot_general(wr8, hn, NT, preferred_element_type=F32)
        r_v[:, rows] = r.astype(BF16).astype(F32)
        out_copy(rows).start()
        return 0
    with _scope('oproj'):
        lax.fori_loop(0, S // OB, oproj, 0)

    r = r_v[0:1, :]
    pos = lax.broadcasted_iota(jnp.int32, (1, S), 1)
    m1 = jnp.max(r, axis=1, keepdims=True)
    i1 = jnp.min(jnp.where(r == m1, pos, S), axis=1, keepdims=True)
    r2 = jnp.where(pos == i1, -jnp.inf, r)
    m2 = jnp.max(r2, axis=1, keepdims=True)
    i2 = jnp.min(jnp.where(r2 == m2, pos, S), axis=1, keepdims=True)
    idx = [jnp.clip(jnp.min(i), 0, S - 1) for i in (i1, i2)]
    sub = lax.broadcasted_iota(jnp.int32, (16, M), 0)
    tiles = [pl.ds(pl.multiple_of((i // 16) * 16, 16), 16) for i in idx]
    sel = [sub == (i % 16) for i in idx]
    xs = [jnp.sum(jnp.where(s, xn_v[t, :].astype(F32), 0.0), axis=0, keepdims=True) for s, t in zip(sel, tiles)]
    x2 = jnp.where(sub == 0, xs[0], jnp.where(sub == 1, xs[1], 0.0)).astype(BF16)
    c_wg.wait(); c_wu.wait(); c_wd.wait()
    g = jnp.dot(x2, wg_v[...], preferred_element_type=F32)
    u = jnp.dot(x2, wu_v[...], preferred_element_type=F32)
    a = (g * jax.nn.sigmoid(g) * u).astype(BF16)
    y = jnp.dot(a, wd_v[...], preferred_element_type=F32)
    out_copy(slice(None)).wait()
    for n, mv in enumerate((m1, m2)):
        yn = y[n:n + 1, :] * jax.nn.sigmoid(mv)
        t = out_ref[tiles[n], :].astype(F32)
        out_ref[tiles[n], :] = jnp.where(sel[n], t + yn, t).astype(BF16)
    out_copy(tiles[0], 9).start()

    @pl.when(idx[0] // 16 != idx[1] // 16)
    def _():
        out_copy(tiles[1], 10).start()
        out_copy(tiles[1], 10).wait()
    out_copy(tiles[0], 9).wait()


@jax.jit
def pallas_sequential_preLN__compressed_kv_cla__moe_arch_mod__prompt_kernel(
    A_x, A_c_kv, A_w_q, A_w_uk, A_w_uv, A_w_o, B_x, B_w_r, B_w_gate, B_w_up, B_w_down,
):
    del B_x
    B, S, M = A_x.shape
    _, H, D = A_w_q.shape
    Dc = A_c_kv.shape[2]
    Fd = B_w_gate.shape[1]
    assert B == 1 and A_c_kv.shape[1] == S
    hbm = pl.BlockSpec(memory_space=pl.ANY)
    vm = lambda shape, dt=BF16: pltpu.VMEM(shape, dt)
    wbuf = lambda m: vm((NPAIRS, 2, m // 2, D), jnp.uint32)
    out = pl.pallas_call(
        functools.partial(_kernel, S=S, M=M, H=H, D=D, Dc=Dc),
        in_specs=[hbm] * 6 + [pl.BlockSpec(memory_space=pltpu.VMEM)] + [hbm] * 3,
        out_specs=hbm,
        out_shape=jax.ShapeDtypeStruct((S, M), BF16),
        scratch_shapes=[
            vm((S, M)), vm((S, Dc)), wbuf(M), wbuf(Dc), wbuf(Dc), vm((H * D, M)),
            vm((M, Fd)), vm((M, Fd)), vm((Fd, M)),
            vm((S, M)), vm((4, S, D)), vm((4, S, D)), vm((H + 1, S, D)), vm((8, S), F32), vm((S, M)),
            pltpu.SMEM((2,), jnp.int32),
            pltpu.SemaphoreType.DMA((11,)), *[pltpu.SemaphoreType.DMA((NPAIRS,))] * 3,
        ],
        compiler_params=pltpu.CompilerParams(vmem_limit_bytes=120 * 1024 * 1024),
    )(
        A_x.reshape(S, M), A_c_kv.reshape(S, Dc), A_w_q.reshape(M // 2, 2 * H, D), A_w_uk.reshape(Dc // 2, 2 * H, D),
        A_w_uv.reshape(Dc // 2, 2 * H, D), A_w_o.reshape(H * D, M), B_w_r.reshape(1, M), B_w_gate, B_w_up, B_w_down,
    )
    return out.reshape(B, S, M)
```

```python
import contextlib
import functools
import math

import jax
import jax.numpy as jnp
from jax import lax
import jax.experimental.pallas as pl
import jax.experimental.pallas.tpu as pltpu

F32 = jnp.float32
BF16 = jnp.bfloat16
EPS = 1e-5
BQ = 2048
BK = 2048
SAFE = 32.0
OB = 256
AHEAD = 4
RB = 256
NPAIRS = 16
NT = (((1,), (1,)), ((), ()))


PROFILE = False


def _scope(name):
    return jax.named_scope(name) if PROFILE else contextlib.nullcontext()


def _fold(x, op):
    r = x[:, :128]
    for c in range(128, x.shape[1], 128):
        r = op(r, x[:, c:c + 128])
    return r


def _recip(x):
    r = pl.reciprocal(x, approx=True)
    return r * (2.0 - x * r)


def _max_sq_norm(x):
    n = jnp.sum(x * x, axis=1, keepdims=True)
    return jnp.max(n)


def _layernorm(x):
    m = jnp.mean(x, axis=-1, keepdims=True)
    d = x - m
    v = jnp.mean(d * d, axis=-1, keepdims=True)
    return d * lax.rsqrt(v + EPS)


def _pair_copies(w_hbm, buf, sems, j):
    w32 = w_hbm.bitcast(jnp.uint32)
    return [pltpu.make_async_copy(w32.at[:, j + e * NPAIRS, :], buf.at[j, e], sems.at[j]) for e in range(2)]


def _pair_weights(buf, j):
    ev, od = buf[j, 0], buf[j, 1]
    lo = (ev & jnp.uint32(0xFFFF)) | (od << 16)
    hi = (ev >> 16) | (od & jnp.uint32(0xFFFF0000))
    return jnp.concatenate([pltpu.bitcast(lo, BF16), pltpu.bitcast(hi, BF16)], axis=1)


def _kernel(x_hbm, ckv_hbm, wq_hbm, wuk_hbm, wuv_hbm, wo_hbm, wr_ref, wg_hbm, wu_hbm, wd_hbm, out_hbm,
            x_v, ckv_v, wq_v, wuk_v, wuv_v, wo_v, wg_v, wu_v, wd_v,
            xn_v, q_v, k_v, v_v, r_v, out_ref, h_v, ok_s, sems, qsem, ksem, vsem, *, S, M, H, D, Dc):
    npairs = H // 2
    cp = lambda i, s, d: pltpu.make_async_copy(s, d, sems.at[i])
    c_x, c_ckv, c_wo = cp(0, x_hbm, x_v), cp(1, ckv_hbm, ckv_v), cp(5, wo_hbm, wo_v)
    q_copies = lambda j: _pair_copies(wq_hbm, wq_v, qsem, j)
    k_copies = lambda j: _pair_copies(wuk_hbm, wuk_v, ksem, j)
    v_copies = lambda j: _pair_copies(wuv_hbm, wuv_v, vsem, j)

    def start(copies):
        for c in copies:
            c.start()

    def wait(copies):
        for c in copies:
            c.wait()
    c_wg, c_wu, c_wd = cp(6, wg_hbm, wg_v), cp(7, wu_hbm, wu_v), cp(8, wd_hbm, wd_v)
    c_ckv.start()
    for j in range(AHEAD):
        start(v_copies(j))
    with _scope('wait_first'):
        c_ckv.wait()
    c_x.start()

    def vproj(j, _):
        if j + AHEAD < NPAIRS:
            start(v_copies(j + AHEAD))
        start(q_copies(j) + k_copies(j))
        wait(v_copies(j))
        v2 = jnp.dot(ckv_v[...], _pair_weights(wuv_v, j), preferred_element_type=F32)
        v_v[2 * j + 1] = v2[:, :D].astype(BF16)
        v_v[2 * j + 2] = v2[:, D:].astype(BF16)
        return 0

    def vproj_ln(j, _):
        vproj(j, 0)
        b = j - (NPAIRS - S // RB)
        rows = pl.ds(b * RB, RB)
        xn_v[rows, :] = _layernorm(x_v[rows, :].astype(F32)).astype(BF16)
        return 0

    with _scope('vproj1'):
        for j in range(NPAIRS - S // RB):
            vproj(j, 0)
    with _scope('wait_x'):
        c_x.wait()
    with _scope('vproj2'):
        for j in range(NPAIRS - S // RB, NPAIRS):
            vproj_ln(j, 0)

    qscale = (D ** -0.5) * math.log2(math.e)
    nq = S // BQ

    def attend(e, h):
        T = 128
        tri = (lax.broadcasted_iota(jnp.int32, (T, T), 1) <= lax.broadcasted_iota(jnp.int32, (T, T), 0))
        nt = BQ // T
        for i in range(nq):
            r0 = i * BQ
            q = q_v[e, r0:r0 + BQ, :]
            pieces = []
            for c0 in range(0, r0, BK):
                c1 = min(c0 + BK, r0)
                pieces.append((0, c0, c1, lax.dot_general(q, k_v[e, c0:c1, :], NT, preferred_element_type=F32)))
            for t in range(nt):
                c0 = r0 + t * T
                sd = lax.dot_general(q[t * T:], k_v[e, c0:c0 + T, :], NT, preferred_element_type=F32)
                top = jnp.where(tri, sd[:T], -1e9)
                sd = top if t == nt - 1 else jnp.concatenate([top, sd[T:]], axis=0)
                pieces.append((t, c0, c0 + T, sd))
            rowtile = lambda a, t0, u: a[(u - t0) * T:(u - t0 + 1) * T]
            o = [None] * nt
            l = [None] * nt
            for t0, c0, c1, sc in pieces:
                p = jnp.exp2(sc)
                pv = jnp.dot(p.astype(BF16), v_v[h + 1, c0:c1, :], preferred_element_type=F32)
                ps = _fold(p, jnp.add)
                for u in range(t0, nt):
                    a, b = rowtile(pv, t0, u), rowtile(ps, t0, u)
                    o[u] = a if o[u] is None else o[u] + a
                    l[u] = b if l[u] is None else l[u] + b
            for u in range(nt):
                ls = jnp.sum(l[u], axis=1, keepdims=True)
                v_v[h, r0 + u * T:r0 + (u + 1) * T, :] = (o[u] * _recip(ls)).astype(BF16)

    def attend_shifted(e, h):
        T = 256
        ri = lax.broadcasted_iota(jnp.int32, (T, T), 0)
        ci = lax.broadcasted_iota(jnp.int32, (T, T), 1)

        def qblock(i, _):
            rows = pl.ds(pl.multiple_of(i * T, T), T)
            q = q_v[e, rows, :]

            def kblock(c, carry):
                m, l, o = carry
                cols = pl.ds(pl.multiple_of(c * T, T), T)
                sc = lax.dot_general(q, k_v[e, cols, :], NT, preferred_element_type=F32)
                sc = jnp.where(ci + c * T <= ri + i * T, sc, -1e9)
                m_new = jnp.maximum(m, jnp.max(sc, axis=1, keepdims=True))
                alpha = jnp.exp2(m - m_new)
                p = jnp.exp2(sc - m_new)
                l = alpha * l + jnp.sum(p, axis=1, keepdims=True)
                o = alpha * o + jnp.dot(p.astype(BF16), v_v[h + 1, cols, :], preferred_element_type=F32)
                return m_new, l, o
            init = (jnp.full((T, 1), -jnp.inf, F32), jnp.zeros((T, 1), F32), jnp.zeros((T, D), F32))
            _, l, o = lax.fori_loop(0, i + 1, kblock, init)
            v_v[h, rows, :] = (o / l).astype(BF16)
            return 0
        lax.fori_loop(0, S // T, qblock, 0)

    def qkproj(j):
        slot = 2 * (j % 2)
        wait(q_copies(j) + k_copies(j))
        q2 = jnp.dot(xn_v[...], _pair_weights(wq_v, j), preferred_element_type=F32) * qscale
        q_v[slot] = q2[:, :D].astype(BF16)
        q_v[slot + 1] = q2[:, D:].astype(BF16)
        k2 = jnp.dot(ckv_v[...], _pair_weights(wuk_v, j), preferred_element_type=F32)
        k_v[slot] = k2[:, :D].astype(BF16)
        k_v[slot + 1] = k2[:, D:].astype(BF16)
        bound = [_max_sq_norm(q2[:, n * D:(n + 1) * D]) * _max_sq_norm(k2[:, n * D:(n + 1) * D])
                 for n in range(2)]
        ok_s[j % 2] = (jnp.maximum(bound[0], bound[1]) <= SAFE * SAFE).astype(jnp.int32)

    qkproj(0)

    def pair(j, _):
        @pl.when(j == 2)
        def _():
            for c in (c_wo, c_wg, c_wu, c_wd):
                c.start()
        pl.when(j + 1 < NPAIRS)(lambda: qkproj(j + 1))
        slot = 2 * (j % 2)
        ok = ok_s[j % 2] == 1

        @pl.when(ok)
        def _():
            with _scope('attn'):
                lax.fori_loop(0, 2, lambda e, c: attend(slot + e, 2 * j + e) or 0, 0)

        @pl.when(jnp.logical_not(ok))
        def _():
            def head(e, _):
                attend_shifted(slot + e, 2 * j + e)
                return 0
            lax.fori_loop(0, 2, head, 0)
        return 0
    with _scope('pairs'):
        lax.fori_loop(0, npairs, pair, 0)

    c_wo.wait()
    wr = wr_ref[...].astype(F32)

    def out_copy(rows, sem=9):
        return pltpu.make_async_copy(out_ref.at[rows], out_hbm.at[rows], sems.at[sem])

    def oproj(b, _):
        r0 = pl.multiple_of(b * OB, OB)
        rows = pl.ds(r0, OB)
        ctx = jnp.concatenate([v_v[h, rows, :] for h in range(H)], axis=1)
        a = jnp.dot(ctx, wo_v[...], preferred_element_type=F32)
        h_v[b % 2] = (x_v[rows, :].astype(F32) + a).astype(BF16)

    def post(b):
        rows = pl.ds(pl.multiple_of(b * OB, OB), OB)
        hh = h_v[b % 2].astype(F32)
        hn = _layernorm(hh).astype(BF16)
        xn_v[rows, :] = hn
        out_ref[rows, :] = (hh + hn.astype(F32)).astype(BF16)
        r = jnp.sum(hn.astype(F32) * wr, axis=1, keepdims=True).astype(BF16).astype(F32)
        lane = lax.broadcasted_iota(jnp.int32, (8, 128), 1)
        dense = jnp.full((8, 128), -jnp.inf, F32)
        for c in range(OB // 8):
            dense = jnp.where(lane == c, r[8 * c:8 * c + 8], dense)
        r_v[b] = dense
        out_copy(rows).start()

    def step(b, _):
        post(b - 1)
        oproj(b, 0)
        return 0
    with _scope('oproj'):
        oproj(0, 0)
        lax.fori_loop(1, S // OB, step, 0)
        post(S // OB - 1)

    nb = S // OB
    r = r_v[...].reshape(nb * 8, 128)
    row = lax.broadcasted_iota(jnp.int32, (nb * 8, 128), 0)
    lane = lax.broadcasted_iota(jnp.int32, (nb * 8, 128), 1)
    pos = jnp.where(lane < OB // 8, (row // 8) * OB + lane * 8 + row % 8, S)
    m1 = jnp.max(r, keepdims=True)
    i1 = jnp.min(jnp.where(r == m1, pos, S), keepdims=True)
    r2 = jnp.where(pos == i1, -jnp.inf, r)
    m2 = jnp.max(r2, keepdims=True)
    i2 = jnp.min(jnp.where((r2 == m2) & (pos != i1), pos, S), keepdims=True)
    idx = [jnp.clip(jnp.min(i), 0, S - 1) for i in (i1, i2)]
    sub = lax.broadcasted_iota(jnp.int32, (16, M), 0)
    tiles = [pl.ds(pl.multiple_of((i // 16) * 16, 16), 16) for i in idx]
    sel = [sub == (i % 16) for i in idx]
    xs = [jnp.sum(jnp.where(s, xn_v[t, :].astype(F32), 0.0), axis=0, keepdims=True) for s, t in zip(sel, tiles)]
    x2 = jnp.where(sub == 0, xs[0], jnp.where(sub == 1, xs[1], 0.0)).astype(BF16)
    c_wg.wait(); c_wu.wait(); c_wd.wait()
    g = jnp.dot(x2, wg_v[...], preferred_element_type=F32)
    u = jnp.dot(x2, wu_v[...], preferred_element_type=F32)
    a = (g * jax.nn.sigmoid(g) * u).astype(BF16)
    y = jnp.dot(a, wd_v[...], preferred_element_type=F32)
    out_copy(slice(None)).wait()
    for n, mv in enumerate((m1, m2)):
        yn = y[n:n + 1, :] * jax.nn.sigmoid(mv)
        t = out_ref[tiles[n], :].astype(F32)
        out_ref[tiles[n], :] = jnp.where(sel[n], t + yn, t).astype(BF16)
    out_copy(tiles[0], 9).start()

    @pl.when(idx[0] // 16 != idx[1] // 16)
    def _():
        out_copy(tiles[1], 10).start()
        out_copy(tiles[1], 10).wait()
    out_copy(tiles[0], 9).wait()


@jax.jit
def pallas_sequential_preLN__compressed_kv_cla__moe_arch_mod__prompt_kernel(
    A_x, A_c_kv, A_w_q, A_w_uk, A_w_uv, A_w_o, B_x, B_w_r, B_w_gate, B_w_up, B_w_down,
):
    del B_x
    B, S, M = A_x.shape
    _, H, D = A_w_q.shape
    Dc = A_c_kv.shape[2]
    Fd = B_w_gate.shape[1]
    assert B == 1 and A_c_kv.shape[1] == S
    hbm = pl.BlockSpec(memory_space=pl.ANY)
    vm = lambda shape, dt=BF16: pltpu.VMEM(shape, dt)
    wbuf = lambda m: vm((NPAIRS, 2, m // 2, D), jnp.uint32)
    out = pl.pallas_call(
        functools.partial(_kernel, S=S, M=M, H=H, D=D, Dc=Dc),
        in_specs=[hbm] * 6 + [pl.BlockSpec(memory_space=pltpu.VMEM)] + [hbm] * 3,
        out_specs=hbm,
        out_shape=jax.ShapeDtypeStruct((S, M), BF16),
        scratch_shapes=[
            vm((S, M)), vm((S, Dc)), wbuf(M), wbuf(Dc), wbuf(Dc), vm((H * D, M)),
            vm((M, Fd)), vm((M, Fd)), vm((Fd, M)),
            vm((S, M)), vm((4, S, D)), vm((4, S, D)), vm((H + 1, S, D)), vm((S // OB, 8, 128), F32), vm((S, M)), vm((2, OB, M)),
            pltpu.SMEM((2,), jnp.int32),
            pltpu.SemaphoreType.DMA((11,)), *[pltpu.SemaphoreType.DMA((NPAIRS,))] * 3,
        ],
        compiler_params=pltpu.CompilerParams(vmem_limit_bytes=120 * 1024 * 1024, flags={"XLA_TPU_EVENLY_DISTRIBUTE_CRITICAL_NODES": True}),
    )(
        A_x.reshape(S, M), A_c_kv.reshape(S, Dc), A_w_q.reshape(M // 2, 2 * H, D), A_w_uk.reshape(Dc // 2, 2 * H, D),
        A_w_uv.reshape(Dc // 2, 2 * H, D), A_w_o.reshape(H * D, M), B_w_r.reshape(1, M), B_w_gate, B_w_up, B_w_down,
    )
    return out.reshape(B, S, M)
```
